```python
import jax
import jax.numpy as jnp

def _softmax(x, axis=-1):
    return jax.nn.softmax(x, axis=axis)
def _gelu(x):
    return jax.nn.gelu(x, approximate=True)
def _silu(x):
    return jax.nn.silu(x)
def _sigmoid(x):
    return jax.nn.sigmoid(x)
def _layernorm(x, axis=-1, eps=1e-5):
    m = jnp.mean(x, axis=axis, keepdims=True)
    v = jnp.var(x, axis=axis, keepdims=True)
    return (x - m) / jnp.sqrt(v + eps)
def _scatter_add(tgt, idx, src, axis=0):
    return tgt.at[idx].add(src)
def _segment_sum(src, seg, n):
    return jax.ops.segment_sum(src, seg, n)
class _Rng:
    def __init__(self, key):
        self._k = key
    def _next(self):
        self._k, sub = jax.random.split(self._k)
        return sub
    def normal(self, shape):
        return jax.random.normal(self._next(), shape, dtype=jnp.bfloat16)
    def randint(self, lo, hi, shape):
        return jax.random.randint(self._next(), shape, lo, hi, dtype=jnp.int32)
    def uniform(self, shape, lo=0.0, hi=1.0):
        return jax.random.uniform(self._next(), shape, jnp.bfloat16, lo, hi)
    def permutation(self, n):
        return jax.random.permutation(self._next(), n)


kernel_name = 'gated_mix__compressed_kv_cla__ssm_conv_s5__prompt'

def setup_inputs():
    _rng = _Rng(jax.random.key(int.from_bytes(__import__("os").urandom(4), "little")))
    _w = (lambda a: (lambda t: t.astype(jnp.bfloat16) if jnp.issubdtype(t.dtype, jnp.floating) else t)(jnp.asarray(a)))
    def _A_setup():
        B, H, Sq, Sk, D, M = 1, 16, 2048, 2048, 256, 448
        Dc = 4 * D
        return {
            "x": _w((lambda *s: _rng.normal(s) * 0.05)(B, Sq, M)),
            "c_kv": _w((lambda *s: _rng.normal(s) * 0.05)(B, Sk, Dc)),
            "w_q": _w((lambda *s: _rng.normal(s) * 0.05)(M, H, D) * (M ** -0.5)),
            "w_uk": _w((lambda *s: _rng.normal(s) * 0.05)(Dc, H, D) * (Dc ** -0.5)),
            "w_uv": _w((lambda *s: _rng.normal(s) * 0.05)(Dc, H, D) * (Dc ** -0.5)),
            "w_o": _w((lambda *s: _rng.normal(s) * 0.05)(H, D, M) * ((H * D) ** -0.5)),
        }
    _A_in = _A_setup()

    def _B_setup():
        B, S, D = 1, 2048, 448
        P = D
        Lambda_re = -0.5 * jnp.exp((lambda *s: _rng.normal(s) * 0.05)(P))
        Lambda_im = (lambda *s: _rng.normal(s) * 0.05)(P) * 1.0
        B_re = (lambda *s: _rng.normal(s) * 0.05)(P, D) * (D ** -0.5)
        B_im = (lambda *s: _rng.normal(s) * 0.05)(P, D) * (D ** -0.5)
        C_re = (lambda *s: _rng.normal(s) * 0.05)(D, P) * (P ** -0.5)
        C_im = (lambda *s: _rng.normal(s) * 0.05)(D, P) * (P ** -0.5)
        log_dt = (lambda *s: _rng.normal(s) * 0.05)(P) * 0.3 - 2.0
        Dskip = (lambda *s: _rng.normal(s) * 0.05)(D)
        return {
            "x": _w((lambda *s: _rng.normal(s) * 0.05)(B, S, D)),
            "Lambda_re": _w(Lambda_re),
            "Lambda_im": _w(Lambda_im),
            "B_re": _w(B_re),
            "B_im": _w(B_im),
            "C_re": _w(C_re),
            "C_im": _w(C_im),
            "log_dt": _w(log_dt),
            "Dskip": _w(Dskip),
        }
    _B_in = _B_setup()

    return {
        "A_x": _A_in["x"],
        "A_c_kv": _A_in["c_kv"],
        "A_w_q": _A_in["w_q"],
        "A_w_uk": _A_in["w_uk"],
        "A_w_uv": _A_in["w_uv"],
        "A_w_o": _A_in["w_o"],
        "B_x": _B_in["x"],
        "B_Lambda_re": _B_in["Lambda_re"],
        "B_Lambda_im": _B_in["Lambda_im"],
        "B_B_re": _B_in["B_re"],
        "B_B_im": _B_in["B_im"],
        "B_C_re": _B_in["C_re"],
        "B_C_im": _B_in["C_im"],
        "B_log_dt": _B_in["log_dt"],
        "B_Dskip": _B_in["Dskip"],
        "gate_w": _w((lambda *s: _rng.normal(s) * 0.05)(448)),
    }

def reference(A_x, A_c_kv, A_w_q, A_w_uk, A_w_uv, A_w_o, B_x, B_Lambda_re, B_Lambda_im, B_B_re, B_B_im, B_C_re, B_C_im, B_log_dt, B_Dskip, gate_w):
    def _A_ref(x, c_kv, w_q, w_uk, w_uv, w_o):
        B, Sq, M = x.shape[0], x.shape[1], x.shape[2]
        Sk = c_kv.shape[1]
        H, D = w_q.shape[1], w_q.shape[2]
        q = jnp.einsum("bqm,mhd->bhqd", x, w_q)
        k = jnp.einsum("bkc,chd->bhkd", c_kv, w_uk)
        v = jnp.einsum("bkc,chd->bhkd", c_kv, w_uv)
        scores = jnp.einsum("bhqd,bhkd->bhqk", q, k) * (D ** -0.5)
        off = Sk - Sq
        qi = jnp.arange(Sq)[:, None]
        kj = jnp.arange(Sk)[None, :]
        cmask = kj <= (qi + off)
        scores = jnp.where(cmask[None, None], scores, -1e9)
        p = _softmax(scores, axis=-1)
        ctx = jnp.einsum("bhqk,bhkd->bhqd", p, v)
        return jnp.einsum("bhqd,hdm->bqm", ctx, w_o)

    def _B_ref(x, Lambda_re, Lambda_im, B_re, B_im, C_re, C_im, log_dt, Dskip):
        Bsz, L, H = x.shape
        Lam = Lambda_re + 1j * Lambda_im
        Bmat = B_re + 1j * B_im
        Cmat = C_re + 1j * C_im
        dt = jnp.exp(log_dt)
        Lam_bar = jnp.exp(dt * Lam)
        B_bar = ((Lam_bar - 1.0) / Lam)[:, None] * Bmat
        Bu = jnp.einsum("bld,pd->blp", x + 0j, B_bar)
        h = jnp.zeros_like(Bu[:, 0, :])
        hs = []
        for t in range(L):
            h = Lam_bar[None, :] * h + Bu[:, t, :]
            hs.append(h)
        hseq = jnp.stack(hs, 1)
        y = 2.0 * jnp.einsum("blp,dp->bld", hseq, Cmat).real + x * Dskip[None, None, :]
        return y

    x = A_x
    g = _sigmoid((x * gate_w).sum(-1, keepdims=True))
    a = _A_ref(x, A_c_kv, A_w_q, A_w_uk, A_w_uv, A_w_o)
    b = _B_ref(x, B_Lambda_re, B_Lambda_im, B_B_re, B_B_im, B_C_re, B_C_im, B_log_dt, B_Dskip)
    return g * a + (1 - g) * b
```

```python
import functools

import jax
import jax.numpy as jnp
import numpy as np
from jax import lax
import jax.experimental.pallas as pl
import jax.experimental.pallas.tpu as pltpu

F32 = jnp.float32
BF16 = jnp.bfloat16
LOG2E = 1.4426950408889634
NT = (((1,), (1,)), ((), ()))


def _dot(a, b):
    return jnp.dot(a, b, preferred_element_type=F32)


def _dot_nt(a, b):
    return lax.dot_general(a, b, NT, preferred_element_type=F32)


def _rb(x):
    return x.astype(BF16).astype(F32)


def _cmul(ar, ai, br, bi):
    return ar * br - ai * bi, ar * bi + ai * br


def _kernel(x_ref, c_ref, wq_hbm, wk_hbm, wv_hbm, wo_ref,
            lre_ref, lim_ref, bre_ref, bim_ref, cre_ref, cim_ref, ldt_ref,
            dsk_ref, gw_ref,
            out_ref,
            lq, lk, lv, wq_s, wk_s, wv_s, q_s, k_s, v_s, acc, hre, him, sems,
            *, S, D, BQ, RC):
    h = pl.program_id(0)
    nh = pl.num_programs(0)

    def copies(j):
        return [
            pltpu.make_async_copy(src.bitcast(jnp.int32).at[:, j, :], dst, sems.at[n])
            for n, (src, dst) in enumerate(((wq_hbm, lq), (wk_hbm, lk), (wv_hbm, lv)))
        ]

    @pl.when(h == 0)
    def _():
        for cp in copies(0):
            cp.start()
        acc[...] = jnp.zeros(acc.shape, F32)

        dt = _rb(jnp.exp(ldt_ref[...].astype(F32)))
        lr = lre_ref[...].astype(F32)
        li = lim_ref[...].astype(F32)
        mag = jnp.exp(dt * lr)
        ar = mag * jnp.cos(dt * li)
        ai = mag * jnp.sin(dt * li)
        den = lr * lr + li * li
        nr = ar - 1.0
        fr = (nr * lr + ai * li) / den
        fi = (ai * lr - nr * li) / den
        P = ar.shape[-1]
        row = lax.broadcasted_iota(jnp.int32, (8, P), 0)
        a1 = (jnp.broadcast_to(ar, (8, P)), jnp.broadcast_to(ai, (8, P)))
        a2 = _cmul(*a1, *a1)
        a4 = _cmul(*a2, *a2)
        a8 = _cmul(*a4, *a4)
        pw = a1
        for s, a in ((1, a1), (2, a2), (4, a4)):
            sel = (row & s) != 0
            t = _cmul(*pw, *a)
            pw = (jnp.where(sel, t[0], pw[0]), jnp.where(sel, t[1], pw[1]))
        steps = [(s, jnp.where(row >= s, a[0], 0.0), jnp.where(row >= s, a[1], 0.0))
                 for s, a in ((1, a1), (2, a2), (4, a4))]

        def proj(i, _):
            r = pl.ds(pl.multiple_of(i * RC, RC), RC)
            xb = x_ref[r, :]
            ur = _dot_nt(xb, bre_ref[...])
            ui = _dot_nt(xb, bim_ref[...])
            hre[r, :] = ur * fr - ui * fi
            him[r, :] = ur * fi + ui * fr
            return 0

        lax.fori_loop(0, S // RC, proj, 0)

        def scan(i, carry):
            cr, ci = carry
            for u in range(8):
                r = pl.ds(pl.multiple_of(i * 64 + u * 8, 8), 8)
                vr = hre[r, :]
                vi = him[r, :]
                for s, mr, mi in steps:
                    sr = pltpu.roll(vr, s, 0)
                    si = pltpu.roll(vi, s, 0)
                    vr, vi = vr + (mr * sr - mi * si), vi + (mr * si + mi * sr)
                vr, vi = vr + (pw[0] * cr - pw[1] * ci), vi + (pw[0] * ci + pw[1] * cr)
                hre[r, :] = vr
                him[r, :] = vi
                cr = jnp.broadcast_to(vr[7:8, :], (8, P))
                ci = jnp.broadcast_to(vi[7:8, :], (8, P))
            return cr, ci

        z = jnp.zeros((8, P), F32)
        lax.fori_loop(0, S // 64, scan, (z, z))

    @pl.when(h % 2 == 0)
    def _():
        j = h // 2
        for cp in copies(j):
            cp.wait()
        for src, dst in ((lq, wq_s), (lk, wk_s), (lv, wv_s)):
            w = src[...]
            dst[0] = pltpu.bitcast(w << 16, F32).astype(BF16)
            dst[1] = pltpu.bitcast(w & jnp.int32(-65536), F32).astype(BF16)

        @pl.when(h + 2 < nh)
        def _():
            for cp in copies(j + 1):
                cp.start()

    par = h % 2
    qscale = (D ** -0.5) * LOG2E

    def proj_qkv(i, _):
        r = pl.ds(pl.multiple_of(i * RC, RC), RC)
        q_s[r, :] = (_dot(x_ref[r, :], wq_s[par]) * qscale).astype(BF16)
        cb = c_ref[r, :]
        k_s[r, :] = _dot(cb, wk_s[par]).astype(BF16)
        v_s[r, :] = _dot(cb, wv_s[par]).astype(BF16)
        return 0

    lax.fori_loop(0, S // RC, proj_qkv, 0)

    tri = (lax.broadcasted_iota(jnp.int32, (BQ, BQ), 0)
           >= lax.broadcasted_iota(jnp.int32, (BQ, BQ), 1))
    for i in range(S // BQ):
        r0 = i * BQ
        q = q_s[r0:r0 + BQ, :]
        sd = jnp.where(tri, _dot_nt(q, k_s[r0:r0 + BQ, :]), -1e9 * LOG2E)
        m = jnp.max(sd, axis=-1, keepdims=True)
        if i > 0:
            so = _dot_nt(q, k_s[0:r0, :])
            m = jnp.maximum(m, jnp.max(so, axis=-1, keepdims=True))
        pd = jnp.exp2(sd - m)
        l = jnp.sum(pd, axis=-1, keepdims=True)
        o = _dot(pd.astype(BF16), v_s[r0:r0 + BQ, :])
        if i > 0:
            po = jnp.exp2(so - m)
            l = l + jnp.sum(po, axis=-1, keepdims=True)
            o = o + _dot(po.astype(BF16), v_s[0:r0, :])
        ctx = (o * (1.0 / l)).astype(BF16)
        acc[r0:r0 + BQ, :] += _dot(ctx, wo_ref[...])

    @pl.when(h == nh - 1)
    def _():
        dsk = dsk_ref[...].astype(F32)
        gw = gw_ref[...].astype(F32)

        def fin(i, _):
            r = pl.ds(pl.multiple_of(i * RC, RC), RC)
            xf = x_ref[r, :].astype(F32)
            y = 2.0 * (_dot_nt(hre[r, :].astype(BF16), cre_ref[...])
                       - _dot_nt(him[r, :].astype(BF16), cim_ref[...]))
            b = y + _rb(xf * dsk)
            z = _rb(jnp.sum(_rb(xf * gw), axis=-1, keepdims=True))
            g = _rb(jax.nn.sigmoid(z))
            out_ref[r, :] = _rb(g * _rb(acc[r, :])) + _rb(1.0 - g) * b
            return 0

        lax.fori_loop(0, S // RC, fin, 0)


@jax.jit
def pallas_gated_mix__compressed_kv_cla__ssm_conv_s5__prompt_kernel(
    A_x: jax.Array,
    A_c_kv: jax.Array,
    A_w_q: jax.Array,
    A_w_uk: jax.Array,
    A_w_uv: jax.Array,
    A_w_o: jax.Array,
    B_x: jax.Array,
    B_Lambda_re: jax.Array,
    B_Lambda_im: jax.Array,
    B_B_re: jax.Array,
    B_B_im: jax.Array,
    B_C_re: jax.Array,
    B_C_im: jax.Array,
    B_log_dt: jax.Array,
    B_Dskip: jax.Array,
    gate_w: jax.Array,
):
    del B_x
    _, S, M = A_x.shape
    Dc = A_c_kv.shape[2]
    H, D = A_w_q.shape[1], A_w_q.shape[2]
    P = B_Lambda_re.shape[0]

    def whole(shape):
        return pl.BlockSpec(shape, lambda h: (0,) * len(shape))

    any_spec = pl.BlockSpec(memory_space=pl.ANY)
    row = lambda v: v.reshape(1, -1)
    out = pl.pallas_call(
        functools.partial(_kernel, S=S, D=D, BQ=256, RC=512),
        grid=(H,),
        in_specs=[
            whole((S, M)), whole((S, Dc)), any_spec, any_spec, any_spec,
            pl.BlockSpec((None, D, M), lambda h: (h, 0, 0)),
            whole((1, P)), whole((1, P)), whole((P, M)), whole((P, M)),
            whole((M, P)), whole((M, P)), whole((1, P)), whole((1, M)), whole((1, M)),
        ],
        out_specs=whole((S, M)),
        out_shape=jax.ShapeDtypeStruct((S, M), F32),
        scratch_shapes=[
            pltpu.VMEM((M, D), jnp.int32), pltpu.VMEM((Dc, D), jnp.int32),
            pltpu.VMEM((Dc, D), jnp.int32),
            pltpu.VMEM((2, M, D), BF16), pltpu.VMEM((2, Dc, D), BF16),
            pltpu.VMEM((2, Dc, D), BF16),
            pltpu.VMEM((S, D), BF16), pltpu.VMEM((S, D), BF16), pltpu.VMEM((S, D), BF16),
            pltpu.VMEM((S, M), F32), pltpu.VMEM((S, P), F32), pltpu.VMEM((S, P), F32),
            pltpu.SemaphoreType.DMA((3,)),
        ],
        compiler_params=pltpu.CompilerParams(
            dimension_semantics=("arbitrary",),
            vmem_limit_bytes=100 * 1024 * 1024,
        ),
    )(A_x.reshape(S, M), A_c_kv.reshape(S, Dc), A_w_q, A_w_uk, A_w_uv, A_w_o,
      row(B_Lambda_re), row(B_Lambda_im), B_B_re, B_B_im, B_C_re, B_C_im,
      row(B_log_dt), row(B_Dskip), row(gate_w))
    return out.reshape(1, S, M)
```

```python
import functools

import jax
import jax.numpy as jnp
import numpy as np
from jax import lax
import jax.experimental.pallas as pl
import jax.experimental.pallas.tpu as pltpu

F32 = jnp.float32
BF16 = jnp.bfloat16
LOG2E = 1.4426950408889634
NT = (((1,), (1,)), ((), ()))


def _dot(a, b):
    return jnp.dot(a, b, preferred_element_type=F32)


def _dot_nt(a, b):
    return lax.dot_general(a, b, NT, preferred_element_type=F32)


def _rb(x):
    return x.astype(BF16).astype(F32)


def _cmul(ar, ai, br, bi):
    return ar * br - ai * bi, ar * bi + ai * br


def _kernel(xt_hbm, c_hbm, wq_hbm, wk_hbm, wv_hbm, wo_ref,
            lre_ref, lim_ref, bre_hbm, bim_hbm, cre_hbm, cim_hbm, ldt_ref,
            dsk_ref, gw_ref,
            out_hbm,
            xt_s, x_s, c_s, bc_s, lq, lk, lv, wq_s, wk_s, wv_s, q_s, k_s, v_s,
            acc, hre, him, sems, isems, osems,
            *, S, D, BQ, RC):
    h = pl.program_id(0)
    nh = pl.num_programs(0)
    M = xt_s.shape[0]

    def copies(j):
        return [
            pltpu.make_async_copy(src.bitcast(jnp.int32).at[:, j, :], dst, sems.at[n])
            for n, (src, dst) in enumerate(((wq_hbm, lq), (wk_hbm, lk), (wv_hbm, lv)))
        ]

    def in_copies():
        pairs = ((xt_hbm, xt_s), (bre_hbm, bc_s.at[0]), (bim_hbm, bc_s.at[1]),
                 (c_hbm, c_s), (cre_hbm, bc_s.at[2]), (cim_hbm, bc_s.at[3]))
        return [pltpu.make_async_copy(a, b, isems.at[n]) for n, (a, b) in enumerate(pairs)]

    @pl.when(h == 0)
    def _():
        ins = in_copies()
        for cp in ins[:4]:
            cp.start()
        for cp in copies(0):
            cp.start()
        for cp in ins[4:]:
            cp.start()
        acc[...] = jnp.zeros(acc.shape, F32)

        row1 = lambda ref: ref[...].astype(F32).reshape(1, -1)
        dt = _rb(jnp.exp(row1(ldt_ref)))
        lr = row1(lre_ref)
        li = row1(lim_ref)
        mag = jnp.exp(dt * lr)
        ar = mag * jnp.cos(dt * li)
        ai = mag * jnp.sin(dt * li)
        den = lr * lr + li * li
        nr = ar - 1.0
        fr = (nr * lr + ai * li) / den
        fi = (ai * lr - nr * li) / den
        P = ar.shape[-1]
        row = lax.broadcasted_iota(jnp.int32, (8, P), 0)
        a1 = (jnp.broadcast_to(ar, (8, P)), jnp.broadcast_to(ai, (8, P)))
        a2 = _cmul(*a1, *a1)
        a4 = _cmul(*a2, *a2)
        pw = a1
        for s, a in ((1, a1), (2, a2), (4, a4)):
            sel = (row & s) != 0
            t = _cmul(*pw, *a)
            pw = (jnp.where(sel, t[0], pw[0]), jnp.where(sel, t[1], pw[1]))
        steps = [(s, jnp.where(row >= s, a[0], 0.0), jnp.where(row >= s, a[1], 0.0))
                 for s, a in ((1, a1), (2, a2), (4, a4))]

        for cp in ins[:3]:
            cp.wait()
        for i in range(S // RC):
            r = slice(i * RC, (i + 1) * RC)
            xb = xt_s[:, r].T
            x_s[r, :] = xb
            ur = _dot_nt(xb, bc_s[0])
            ui = _dot_nt(xb, bc_s[1])
            hre[r, :] = ur * fr - ui * fi
            him[r, :] = ur * fi + ui * fr

        def scan(i, carry):
            cr, ci = carry
            for u in range(8):
                r = pl.ds(pl.multiple_of(i * 64 + u * 8, 8), 8)
                vr = hre[r, :]
                vi = him[r, :]
                for s, mr, mi in steps:
                    sr = pltpu.roll(vr, s, 0)
                    si = pltpu.roll(vi, s, 0)
                    vr, vi = vr + (mr * sr - mi * si), vi + (mr * si + mi * sr)
                vr, vi = vr + (pw[0] * cr - pw[1] * ci), vi + (pw[0] * ci + pw[1] * cr)
                hre[r, :] = vr
                him[r, :] = vi
                cr = jnp.broadcast_to(vr[7:8, :], (8, P))
                ci = jnp.broadcast_to(vi[7:8, :], (8, P))
            return cr, ci

        z = jnp.zeros((8, P), F32)
        lax.fori_loop(0, S // 64, scan, (z, z))
        for cp in ins[3:]:
            cp.wait()

    @pl.when(h % 2 == 0)
    def _():
        j = h // 2
        for cp in copies(j):
            cp.wait()
        for src, dst in ((lq, wq_s), (lk, wk_s), (lv, wv_s)):
            w = src[...]
            dst[0] = pltpu.bitcast(w << 16, F32).astype(BF16)
            dst[1] = pltpu.bitcast(w & jnp.int32(-65536), F32).astype(BF16)

        @pl.when(h + 2 < nh)
        def _():
            for cp in copies(j + 1):
                cp.start()

    par = h % 2
    qscale = (D ** -0.5) * LOG2E

    def proj_qkv(i, _):
        r = pl.ds(pl.multiple_of(i * RC, RC), RC)
        q_s[r, :] = (_dot(x_s[r, :], wq_s[par]) * qscale).astype(BF16)
        cb = c_s[r, :]
        k_s[r, :] = _dot(cb, wk_s[par]).astype(BF16)
        v_s[r, :] = _dot(cb, wv_s[par]).astype(BF16)
        return 0

    lax.fori_loop(0, S // RC, proj_qkv, 0)

    T = 128
    tri = (lax.broadcasted_iota(jnp.int32, (T, T), 0)
           >= lax.broadcasted_iota(jnp.int32, (T, T), 1))
    NEG = -1e9 * LOG2E
    nt = BQ // T
    for i in range(S // BQ):
        r0 = i * BQ
        q = q_s[r0:r0 + BQ, :]
        s0 = _dot_nt(q, k_s[0:r0 + T, :])
        sj = [_dot_nt(q[j * T:, :], k_s[r0 + j * T:r0 + (j + 1) * T, :]) for j in range(1, nt)]
        p0, pj, ls = [], [[] for _ in range(1, nt)], []
        for a in range(nt):
            parts = [s0[a * T:(a + 1) * T, :]]
            for j in range(1, a + 1):
                parts.append(sj[j - 1][(a - j) * T:(a - j + 1) * T, :])
            n = parts[-1].shape[1]
            last = jnp.where(tri, parts[-1][:, n - T:], NEG)
            parts[-1] = last if n == T else jnp.concatenate([parts[-1][:, :n - T], last], axis=1)
            srow = parts[0] if a == 0 else jnp.concatenate(parts, axis=1)
            m = jnp.max(srow, axis=-1, keepdims=True)
            p = jnp.exp2(srow - m)
            ls.append(jnp.sum(p, axis=-1, keepdims=True))
            p = p.astype(BF16)
            p0.append(p[:, :r0 + T])
            for j in range(1, a + 1):
                pj[j - 1].append(p[:, r0 + j * T:r0 + (j + 1) * T])
        o = _dot(jnp.concatenate(p0, axis=0), v_s[0:r0 + T, :])
        oj = [_dot(jnp.concatenate(pj[j - 1], axis=0), v_s[r0 + j * T:r0 + (j + 1) * T, :])
              for j in range(1, nt)]
        ctx = []
        for a in range(nt):
            oa = o[a * T:(a + 1) * T, :]
            for j in range(1, a + 1):
                oa = oa + oj[j - 1][(a - j) * T:(a - j + 1) * T, :]
            ctx.append((oa * (1.0 / ls[a])).astype(BF16))
        ctx = jnp.concatenate(ctx, axis=0)
        acc[:, r0:r0 + BQ] += _dot_nt(wo_ref[...], ctx)

    @pl.when(h == nh - 1)
    def _():
        def col(ref):
            v = jnp.broadcast_to(ref[...].astype(F32).reshape(1, -1), (T, M))
            return v.T[:, :1]
        dsk = col(dsk_ref)
        gw = col(gw_ref)
        outs = []
        for i in range(S // RC):
            r = slice(i * RC, (i + 1) * RC)
            xf = xt_s[:, r].astype(F32)
            y = 2.0 * (_dot_nt(bc_s[2], hre[r, :].astype(BF16))
                       - _dot_nt(bc_s[3], him[r, :].astype(BF16)))
            b = y + _rb(xf * dsk)
            z = _rb(jnp.sum(_rb(xf * gw), axis=0, keepdims=True))
            g = _rb(jax.nn.sigmoid(z))
            acc[:, r] = _rb(g * _rb(acc[:, r])) + _rb(1.0 - g) * b
            cp = pltpu.make_async_copy(acc.at[:, r], out_hbm.at[:, r], osems.at[i])
            cp.start()
            outs.append(cp)
        for cp in outs:
            cp.wait()


@jax.jit
def pallas_gated_mix__compressed_kv_cla__ssm_conv_s5__prompt_kernel(
    A_x: jax.Array,
    A_c_kv: jax.Array,
    A_w_q: jax.Array,
    A_w_uk: jax.Array,
    A_w_uv: jax.Array,
    A_w_o: jax.Array,
    B_x: jax.Array,
    B_Lambda_re: jax.Array,
    B_Lambda_im: jax.Array,
    B_B_re: jax.Array,
    B_B_im: jax.Array,
    B_C_re: jax.Array,
    B_C_im: jax.Array,
    B_log_dt: jax.Array,
    B_Dskip: jax.Array,
    gate_w: jax.Array,
):
    del B_x
    _, S, M = A_x.shape
    Dc = A_c_kv.shape[2]
    H, D = A_w_q.shape[1], A_w_q.shape[2]
    P = B_Lambda_re.shape[0]
    assert P == M
    RC = 512

    hbm = pl.BlockSpec(memory_space=pltpu.HBM)
    vec = pl.BlockSpec((M,), lambda h: (0,))
    out_t = pl.pallas_call(
        functools.partial(_kernel, S=S, D=D, BQ=512, RC=RC),
        grid=(H,),
        in_specs=[
            hbm, hbm, hbm, hbm, hbm,
            pl.BlockSpec((None, M, D), lambda h: (h, 0, 0)),
            vec, vec, hbm, hbm, hbm, hbm, vec, vec, vec,
        ],
        out_specs=hbm,
        out_shape=jax.ShapeDtypeStruct((M, S), F32),
        scratch_shapes=[
            pltpu.VMEM((M, S), BF16), pltpu.VMEM((S, M), BF16), pltpu.VMEM((S, Dc), BF16),
            pltpu.VMEM((4, M, M), BF16),
            pltpu.VMEM((M, D), jnp.int32), pltpu.VMEM((Dc, D), jnp.int32),
            pltpu.VMEM((Dc, D), jnp.int32),
            pltpu.VMEM((2, M, D), BF16), pltpu.VMEM((2, Dc, D), BF16),
            pltpu.VMEM((2, Dc, D), BF16),
            pltpu.VMEM((S, D), BF16), pltpu.VMEM((S, D), BF16), pltpu.VMEM((S, D), BF16),
            pltpu.VMEM((M, S), F32), pltpu.VMEM((S, P), F32), pltpu.VMEM((S, P), F32),
            pltpu.SemaphoreType.DMA((3,)), pltpu.SemaphoreType.DMA((6,)),
            pltpu.SemaphoreType.DMA((S // RC,)),
        ],
        compiler_params=pltpu.CompilerParams(
            dimension_semantics=("arbitrary",),
            vmem_limit_bytes=100 * 1024 * 1024,
        ),
    )(A_x.reshape(S, M).T, A_c_kv.reshape(S, Dc), A_w_q, A_w_uk, A_w_uv,
      jnp.swapaxes(A_w_o, 1, 2),
      B_Lambda_re, B_Lambda_im, B_B_re, B_B_im, B_C_re, B_C_im,
      B_log_dt, B_Dskip, gate_w)
    return out_t.T.reshape(1, S, M)
```

```python
import functools

import jax
import jax.numpy as jnp
import numpy as np
from jax import lax
import jax.experimental.pallas as pl
import jax.experimental.pallas.tpu as pltpu

F32 = jnp.float32
BF16 = jnp.bfloat16
LOG2E = 1.4426950408889634
KCHUNK = 256
PIPE = 1
NT = (((1,), (1,)), ((), ()))


def _dot(a, b):
    return jnp.dot(a, b, preferred_element_type=F32)


def _dot_nt(a, b):
    return lax.dot_general(a, b, NT, preferred_element_type=F32)


def _rb(x):
    return x.astype(BF16).astype(F32)


def _cmul(ar, ai, br, bi):
    return ar * br - ai * bi, ar * bi + ai * br


def _kernel(xt_hbm, c_hbm, wq_hbm, wk_hbm, wv_hbm, wo_ref,
            lre_ref, lim_ref, bre_hbm, bim_hbm, cre_hbm, cim_hbm, ldt_ref,
            dsk_ref, gw_ref,
            out_hbm,
            xt_s, x_s, c_s, bc_s, lq, lk, lv, wq_s, wk_s, wv_s, q_s, k_s, v_s,
            acc, hre, him, sems, isems, osems,
            *, S, D, BQ, RC):
    h = pl.program_id(0)
    nh = pl.num_programs(0)
    M = xt_s.shape[0]

    def copies(j):
        return [
            pltpu.make_async_copy(src.bitcast(jnp.int32).at[:, j, :], dst, sems.at[n])
            for n, (src, dst) in enumerate(((wq_hbm, lq), (wk_hbm, lk), (wv_hbm, lv)))
        ]

    def in_copies():
        pairs = ((xt_hbm, xt_s), (bre_hbm, bc_s.at[0]), (bim_hbm, bc_s.at[1]),
                 (c_hbm, c_s), (cre_hbm, bc_s.at[2]), (cim_hbm, bc_s.at[3]))
        return [pltpu.make_async_copy(a, b, isems.at[n]) for n, (a, b) in enumerate(pairs)]

    @pl.when(h == 0)
    def _():
        ins = in_copies()
        for cp in ins[:4]:
            cp.start()
        for cp in copies(0):
            cp.start()
        for cp in ins[4:]:
            cp.start()
        acc[...] = jnp.zeros(acc.shape, F32)

        row1 = lambda ref: ref[...].astype(F32).reshape(1, -1)
        dt = _rb(jnp.exp(row1(ldt_ref)))
        lr = row1(lre_ref)
        li = row1(lim_ref)
        mag = jnp.exp(dt * lr)
        ar = mag * jnp.cos(dt * li)
        ai = mag * jnp.sin(dt * li)
        den = lr * lr + li * li
        nr = ar - 1.0
        fr = (nr * lr + ai * li) / den
        fi = (ai * lr - nr * li) / den
        P = ar.shape[-1]
        row = lax.broadcasted_iota(jnp.int32, (8, P), 0)
        a1 = (jnp.broadcast_to(ar, (8, P)), jnp.broadcast_to(ai, (8, P)))
        a2 = _cmul(*a1, *a1)
        a4 = _cmul(*a2, *a2)
        pw = a1
        for s, a in ((1, a1), (2, a2), (4, a4)):
            sel = (row & s) != 0
            t = _cmul(*pw, *a)
            pw = (jnp.where(sel, t[0], pw[0]), jnp.where(sel, t[1], pw[1]))
        steps = [(s, jnp.where(row >= s, a[0], 0.0), jnp.where(row >= s, a[1], 0.0))
                 for s, a in ((1, a1), (2, a2), (4, a4))]

        for cp in ins[:3]:
            cp.wait()
        for i in range(S // RC):
            r = slice(i * RC, (i + 1) * RC)
            xb = xt_s[:, r].T
            x_s[r, :] = xb
            ur = _dot_nt(xb, bc_s[0])
            ui = _dot_nt(xb, bc_s[1])
            hre[r, :] = ur * fr - ui * fi
            him[r, :] = ur * fi + ui * fr

        def scan(i, carry):
            cr, ci = carry
            for u in range(8):
                r = pl.ds(pl.multiple_of(i * 64 + u * 8, 8), 8)
                vr = hre[r, :]
                vi = him[r, :]
                for s, mr, mi in steps:
                    sr = pltpu.roll(vr, s, 0)
                    si = pltpu.roll(vi, s, 0)
                    vr, vi = vr + (mr * sr - mi * si), vi + (mr * si + mi * sr)
                vr, vi = vr + (pw[0] * cr - pw[1] * ci), vi + (pw[0] * ci + pw[1] * cr)
                hre[r, :] = vr
                him[r, :] = vi
                cr = jnp.broadcast_to(vr[7:8, :], (8, P))
                ci = jnp.broadcast_to(vi[7:8, :], (8, P))
            return cr, ci

        z = jnp.zeros((8, P), F32)
        lax.fori_loop(0, S // 64, scan, (z, z))
        for cp in ins[3:]:
            cp.wait()

    @pl.when(h % 2 == 0)
    def _():
        j = h // 2
        for cp in copies(j):
            cp.wait()
        for src, dst in ((lq, wq_s), (lk, wk_s), (lv, wv_s)):
            w = src[...]
            dst[0] = pltpu.bitcast(w << 16, F32).astype(BF16)
            dst[1] = pltpu.bitcast(w & jnp.int32(-65536), F32).astype(BF16)

        @pl.when(h + 2 < nh)
        def _():
            for cp in copies(j + 1):
                cp.start()

    par = h % 2
    qscale = (D ** -0.5) * LOG2E

    def proj_qkv(i, _):
        r = pl.ds(pl.multiple_of(i * RC, RC), RC)
        q_s[r, :] = (_dot(x_s[r, :], wq_s[par]) * qscale).astype(BF16)
        cb = c_s[r, :]
        k_s[r, :] = _dot(cb, wk_s[par]).astype(BF16)
        v_s[r, :] = _dot(cb, wv_s[par]).astype(BF16)
        return 0

    lax.fori_loop(0, S // RC, proj_qkv, 0)

    T = 128
    KC = KCHUNK
    tri = (lax.broadcasted_iota(jnp.int32, (T, T), 0)
           >= lax.broadcasted_iota(jnp.int32, (T, T), 1))
    NEG = -1e9 * LOG2E
    nt = BQ // T

    def lane_fold(v, op):
        r = v[:, :T]
        for t in range(1, v.shape[1] // T):
            r = op(r, v[:, t * T:(t + 1) * T])
        return r

    def pad_top(v, j, fill):
        return v if j == 0 else jnp.concatenate([jnp.full((j * T, v.shape[1]), fill, F32), v], axis=0)

    def key_parts(i):
        r0 = i * BQ
        return ([(0, k0, k0 + KC) for k0 in range(0, r0, KC)]
                + [(j, r0 + j * T, r0 + (j + 1) * T) for j in range(nt)])

    units = [(i, k0) for i in range(S // BQ) for k0 in [None] + list(range(0, i * BQ, KC))]

    def qk(i, k0):
        r0 = i * BQ
        if k0 is not None:
            return _dot_nt(q_s[r0:r0 + BQ, :], k_s[k0:k0 + KC, :])
        out = []
        for j in range(nt):
            s = _dot_nt(q_s[r0 + j * T:r0 + BQ, :], k_s[r0 + j * T:r0 + (j + 1) * T, :])
            top = jnp.where(tri, s[:T], NEG)
            out.append(top if j == nt - 1 else jnp.concatenate([top, s[T:]], axis=0))
        return out

    def chain(parts, op):
        r = parts[0]
        for j in range(1, nt):
            r = jnp.concatenate([r[:j * T], op(r[j * T:], parts[j])], axis=0)
        return r

    pend = [qk(*units[n]) for n in range(PIPE)]
    for n, (i, k0) in enumerate(units):
        r0 = i * BQ
        if n + PIPE < len(units):
            pend.append(qk(*units[n + PIPE]))
        s = pend.pop(0)
        if k0 is None:
            m = jnp.max(chain(s, jnp.maximum), axis=-1, keepdims=True)
            p = [jnp.exp2(s[j] - m[j * T:]) for j in range(nt)]
            l = chain(p, jnp.add)
            o = chain([_dot(p[j].astype(BF16), v_s[r0 + j * T:r0 + (j + 1) * T, :])
                       for j in range(nt)], jnp.add)
        else:
            mn = jnp.maximum(m, jnp.max(lane_fold(s, jnp.maximum), axis=-1, keepdims=True))
            al = jnp.exp2(m - mn)
            m = mn
            p = jnp.exp2(s - m)
            l = l * al + lane_fold(p, jnp.add)
            o = o * al + _dot(p.astype(BF16), v_s[k0:k0 + KC, :])
        if n + 1 == len(units) or units[n + 1][1] is None:
            ctx = (o * (1.0 / jnp.sum(l, axis=-1, keepdims=True))).astype(BF16)
            acc[:, r0:r0 + BQ] += _dot_nt(wo_ref[...], ctx)

    @pl.when(h == nh - 1)
    def _():
        def col(ref):
            v = jnp.broadcast_to(ref[...].astype(F32).reshape(1, -1), (T, M))
            return v.T[:, :1]
        dsk = col(dsk_ref)
        gw = col(gw_ref)
        outs = []
        for i in range(S // RC):
            r = slice(i * RC, (i + 1) * RC)
            xf = xt_s[:, r].astype(F32)
            y = 2.0 * (_dot_nt(bc_s[2], hre[r, :].astype(BF16))
                       - _dot_nt(bc_s[3], him[r, :].astype(BF16)))
            b = y + _rb(xf * dsk)
            z = _rb(jnp.sum(_rb(xf * gw), axis=0, keepdims=True))
            g = _rb(jax.nn.sigmoid(z))
            acc[:, r] = _rb(g * _rb(acc[:, r])) + _rb(1.0 - g) * b
            cp = pltpu.make_async_copy(acc.at[:, r], out_hbm.at[:, r], osems.at[i])
            cp.start()
            outs.append(cp)
        for cp in outs:
            cp.wait()


@jax.jit
def pallas_gated_mix__compressed_kv_cla__ssm_conv_s5__prompt_kernel(
    A_x: jax.Array,
    A_c_kv: jax.Array,
    A_w_q: jax.Array,
    A_w_uk: jax.Array,
    A_w_uv: jax.Array,
    A_w_o: jax.Array,
    B_x: jax.Array,
    B_Lambda_re: jax.Array,
    B_Lambda_im: jax.Array,
    B_B_re: jax.Array,
    B_B_im: jax.Array,
    B_C_re: jax.Array,
    B_C_im: jax.Array,
    B_log_dt: jax.Array,
    B_Dskip: jax.Array,
    gate_w: jax.Array,
):
    del B_x
    _, S, M = A_x.shape
    Dc = A_c_kv.shape[2]
    H, D = A_w_q.shape[1], A_w_q.shape[2]
    P = B_Lambda_re.shape[0]
    assert P == M
    RC = 512

    hbm = pl.BlockSpec(memory_space=pltpu.HBM)
    vec = pl.BlockSpec((M,), lambda h: (0,))
    out_t = pl.pallas_call(
        functools.partial(_kernel, S=S, D=D, BQ=512, RC=RC),
        grid=(H,),
        in_specs=[
            hbm, hbm, hbm, hbm, hbm,
            pl.BlockSpec((None, M, D), lambda h: (h, 0, 0)),
            vec, vec, hbm, hbm, hbm, hbm, vec, vec, vec,
        ],
        out_specs=hbm,
        out_shape=jax.ShapeDtypeStruct((M, S), F32),
        scratch_shapes=[
            pltpu.VMEM((M, S), BF16), pltpu.VMEM((S, M), BF16), pltpu.VMEM((S, Dc), BF16),
            pltpu.VMEM((4, M, M), BF16),
            pltpu.VMEM((M, D), jnp.int32), pltpu.VMEM((Dc, D), jnp.int32),
            pltpu.VMEM((Dc, D), jnp.int32),
            pltpu.VMEM((2, M, D), BF16), pltpu.VMEM((2, Dc, D), BF16),
            pltpu.VMEM((2, Dc, D), BF16),
            pltpu.VMEM((S, D), BF16), pltpu.VMEM((S, D), BF16), pltpu.VMEM((S, D), BF16),
            pltpu.VMEM((M, S), F32), pltpu.VMEM((S, P), F32), pltpu.VMEM((S, P), F32),
            pltpu.SemaphoreType.DMA((3,)), pltpu.SemaphoreType.DMA((6,)),
            pltpu.SemaphoreType.DMA((S // RC,)),
        ],
        compiler_params=pltpu.CompilerParams(
            dimension_semantics=("arbitrary",),
            vmem_limit_bytes=100 * 1024 * 1024,
        ),
    )(A_x.reshape(S, M).T, A_c_kv.reshape(S, Dc), A_w_q, A_w_uk, A_w_uv,
      jnp.swapaxes(A_w_o, 1, 2),
      B_Lambda_re, B_Lambda_im, B_B_re, B_B_im, B_C_re, B_C_im,
      B_log_dt, B_Dskip, gate_w)
    return out_t.T.reshape(1, S, M)
```

```python
import functools

import jax
import jax.numpy as jnp
import numpy as np
from jax import lax
import jax.experimental.pallas as pl
import jax.experimental.pallas.tpu as pltpu

F32 = jnp.float32
BF16 = jnp.bfloat16
LOG2E = 1.4426950408889634
KCHUNK = 256
NT = (((1,), (1,)), ((), ()))


def _dot(a, b):
    return jnp.dot(a, b, preferred_element_type=F32)


def _dot_nt(a, b):
    return lax.dot_general(a, b, NT, preferred_element_type=F32)


def _rb(x):
    return x.astype(BF16).astype(F32)


def _cmul(ar, ai, br, bi):
    return ar * br - ai * bi, ar * bi + ai * br


def _kernel(xt_hbm, c_hbm, wq_hbm, wk_hbm, wv_hbm, wo_ref,
            lre_ref, lim_ref, bre_hbm, bim_hbm, cre_hbm, cim_hbm, ldt_ref,
            dsk_ref, gw_ref,
            out_hbm,
            xt_s, x_s, c_s, bc_s, lq, lk, lv, wq_s, wk_s, wv_s, q_s, k_s, v_s,
            acc, hre, him, sems, isems, osems,
            *, S, D, BQ, RC, NH):
    h = pl.program_id(0)
    nh = pl.num_programs(0)
    M = xt_s.shape[0]

    def copies(j):
        return [
            pltpu.make_async_copy(src.bitcast(jnp.int32).at[:, j, :], dst.at[j % 2],
                                  sems.at[n])
            for n, (src, dst) in enumerate(((wq_hbm, lq), (wk_hbm, lk), (wv_hbm, lv)))
        ]

    def in_copy(n):
        pairs = ((xt_hbm, xt_s), (bre_hbm, bc_s.at[0]), (bim_hbm, bc_s.at[1]),
                 (c_hbm, c_s), (cre_hbm, bc_s.at[2]), (cim_hbm, bc_s.at[3]))
        return pltpu.make_async_copy(*pairs[n], isems.at[n])

    def unpack(hn, which=(0, 1, 2)):
        sh = 16 - 16 * (hn % 2)
        for src, dst in [((lq, wq_s), (lk, wk_s), (lv, wv_s))[w] for w in which]:
            w = (src[(hn // 2) % 2] << sh) & jnp.int32(-65536)
            dst[hn % 2] = pltpu.bitcast(w, F32).astype(BF16)

    @pl.when(h == 0)
    def _():
        ins = [in_copy(n) for n in range(6)]
        for cp in ins[:4]:
            cp.start()
        for cp in copies(0):
            cp.start()
        for cp in ins[4:]:
            cp.start()
        acc[...] = jnp.zeros(acc.shape, F32)

        row1 = lambda ref: ref[...].astype(F32).reshape(1, -1)
        dt = _rb(jnp.exp(row1(ldt_ref)))
        lr = row1(lre_ref)
        li = row1(lim_ref)
        mag = jnp.exp(dt * lr)
        ar = mag * jnp.cos(dt * li)
        ai = mag * jnp.sin(dt * li)
        den = lr * lr + li * li
        nr = ar - 1.0
        fr = (nr * lr + ai * li) / den
        fi = (ai * lr - nr * li) / den
        P = ar.shape[-1]
        seg = S // 8
        NL = hre.shape[0]

        def tiles(v):
            v = jnp.concatenate([v, jnp.zeros((v.shape[0], NL * 128 - P), F32)], axis=1)
            return [v[:, t * 128:(t + 1) * 128] for t in range(NL)]

        a1 = tuple(jnp.stack(tiles(jnp.broadcast_to(v, (8, P)))) for v in (ar, ai))

        for cp in ins[:3]:
            cp.wait()

        @pl.loop(0, S // RC)
        def _(i):
            r = pl.ds(pl.multiple_of(i * RC, RC), RC)
            xb = xt_s[:, r].T
            x_s[r, :] = xb
            ur = _dot_nt(xb, bc_s[0])
            ui = _dot_nt(xb, bc_s[1])
            vr = tiles(ur * fr - ui * fi)
            vi = tiles(ur * fi + ui * fr)
            for u in range(RC // seg):
                d = pl.ds(i * (RC // seg) + u, seg, stride=8)
                for t in range(NL):
                    hre[t, d, :] = vr[t][u * seg:(u + 1) * seg]
                    him[t, d, :] = vi[t][u * seg:(u + 1) * seg]

        def sweep(init, store):
            def body(i, st):
                for u in range(8):
                    r = pl.ds(pl.multiple_of(i * 64 + u * 8, 8), 8)
                    pr, pi = _cmul(*a1, *st)
                    st = (hre[:, r, :] + pr, him[:, r, :] + pi)
                    if store:
                        hre[:, r, :] = st[0]
                        him[:, r, :] = st[1]
                return st
            return lax.fori_loop(0, seg // 8, body, init)

        z = jnp.zeros((NL, 8, 128), F32)
        er, ei = sweep((z, z), False)
        al = a1
        for _ in range(seg.bit_length() - 1):
            al = _cmul(*al, *al)
        row = lax.broadcasted_iota(jnp.int32, z.shape, 1)
        sr, si = z, z
        for _ in range(7):
            pr, pi = _cmul(*al, sr, si)
            sr = jnp.where(row > 0, pltpu.roll(er + pr, 1, 1), 0.0)
            si = jnp.where(row > 0, pltpu.roll(ei + pi, 1, 1), 0.0)
        sweep((sr, si), True)
        ins[3].wait()
        for cp in copies(0):
            cp.wait()
        unpack(0)

    @pl.when(jnp.logical_and(h % 2 == 0, h + 2 < nh))
    def _():
        for cp in copies(h // 2 + 1):
            cp.start()

    @pl.when(jnp.logical_and(h % 2 == 1, h + 1 < nh))
    def _():
        for cp in copies(h // 2 + 1):
            cp.wait()

    par = h % 2
    qscale = (D ** -0.5) * LOG2E

    def proj(i):
        r = slice(i * BQ, (i + 1) * BQ)
        q_s[r, :] = (_dot(x_s[r, :], wq_s[par]) * qscale).astype(BF16)
        cb = c_s[r, :]
        k_s[r, :] = _dot(cb, wk_s[par]).astype(BF16)
        v_s[r, :] = _dot(cb, wv_s[par]).astype(BF16)

    T = 128
    KC = KCHUNK
    tri = (lax.broadcasted_iota(jnp.int32, (T, T), 0)
           >= lax.broadcasted_iota(jnp.int32, (T, T), 1))
    NEG = -1e9 * LOG2E
    nt = BQ // T

    def lane_fold(v, op):
        r = v[:, :T]
        for t in range(1, v.shape[1] // T):
            r = op(r, v[:, t * T:(t + 1) * T])
        return r

    def pad_top(v, j, fill):
        return v if j == 0 else jnp.concatenate([jnp.full((j * T, v.shape[1]), fill, F32), v], axis=0)

    def key_parts(i):
        r0 = i * BQ
        return ([(0, k0, k0 + KC) for k0 in range(0, r0, KC)]
                + [(j, r0 + j * T, r0 + (j + 1) * T) for j in range(nt)])

    units = [(i, k0) for i in range(S // BQ) for k0 in [None] + list(range(0, i * BQ, KC))]

    def qk(i, k0):
        r0 = i * BQ
        if k0 is not None:
            return _dot_nt(q_s[r0:r0 + BQ, :], k_s[k0:k0 + KC, :])
        out = []
        for j in range(nt):
            s = _dot_nt(q_s[r0 + j * T:r0 + BQ, :], k_s[r0 + j * T:r0 + (j + 1) * T, :])
            top = jnp.where(tri, s[:T], NEG)
            out.append(top if j == nt - 1 else jnp.concatenate([top, s[T:]], axis=0))
        return out

    def chain(parts, op):
        r = parts[0]
        for j in range(1, nt):
            r = jnp.concatenate([r[:j * T], op(r[j * T:], parts[j])], axis=0)
        return r

    def wo(i, ctx):
        acc[:, i * BQ:(i + 1) * BQ] += _dot_nt(wo_ref[...], ctx)

    @pl.when(h >= 0)
    def _():
        unpack(h + 1)
    proj(0)
    pend = [qk(*units[0])]
    late = []
    for n, (i, k0) in enumerate(units):
        r0 = i * BQ
        if n + 1 < len(units):
            if units[n + 1][1] is None:
                proj(i + 1)
            pend.append(qk(*units[n + 1]))
        s = pend.pop(0)
        if k0 is None:
            m = jnp.max(chain(s, jnp.maximum), axis=-1, keepdims=True)
            p = [jnp.exp2(s[j] - m[j * T:]) for j in range(nt)]
            l = chain(p, jnp.add)
            o = chain([_dot(p[j].astype(BF16), v_s[r0 + j * T:r0 + (j + 1) * T, :])
                       for j in range(nt)], jnp.add)
        else:
            mn = jnp.maximum(m, jnp.max(lane_fold(s, jnp.maximum), axis=-1, keepdims=True))
            al = jnp.exp2(m - mn)
            m = mn
            p = jnp.exp2(s - m)
            l = l * al + lane_fold(p, jnp.add)
            o = o * al + _dot(p.astype(BF16), v_s[k0:k0 + KC, :])
        if n + 1 == len(units) or units[n + 1][1] is None:
            ctx = (o * (1.0 / jnp.sum(l, axis=-1, keepdims=True))).astype(BF16)
            late.append((i, ctx))
            if i < 3:
                wo(*late.pop(0))
    for it in late:
        wo(*it)

    @pl.when(h == nh - 1)
    def _():
        def col(ref):
            v = jnp.broadcast_to(ref[...].astype(F32).reshape(1, -1), (T, M))
            return v.T[:, :1]
        dsk = col(dsk_ref)
        gw = col(gw_ref)
        in_copy(4).wait()
        in_copy(5).wait()

        def out_copy(i):
            r = pl.ds(pl.multiple_of(i * RC, RC), RC)
            return pltpu.make_async_copy(acc.at[:, r], out_hbm.at[:, r], osems.at[i])

        @pl.loop(0, S // RC)
        def _(i):
            r = pl.ds(pl.multiple_of(i * RC, RC), RC)
            xf = xt_s[:, r].astype(F32)
            seg = S // 8
            hr, hi = [
                jnp.concatenate([
                    jnp.concatenate([ref[t, pl.ds(i * (RC // seg) + u, seg, stride=8), :]
                                     for t in range(ref.shape[0])], axis=1)
                    for u in range(RC // seg)], axis=0)[:, :M].astype(BF16)
                for ref in (hre, him)]
            b = 2.0 * (_dot_nt(bc_s[2], hr) - _dot_nt(bc_s[3], hi)) + _rb(xf * dsk)
            z = _rb(jnp.sum(_rb(xf * gw), axis=0, keepdims=True))
            g = _rb(jax.nn.sigmoid(z))
            acc[:, r] = _rb(g * _rb(acc[:, r])) + _rb(1.0 - g) * b
            out_copy(i).start()

        for i in range(S // RC):
            out_copy(i).wait()


@jax.jit
def pallas_gated_mix__compressed_kv_cla__ssm_conv_s5__prompt_kernel(
    A_x: jax.Array,
    A_c_kv: jax.Array,
    A_w_q: jax.Array,
    A_w_uk: jax.Array,
    A_w_uv: jax.Array,
    A_w_o: jax.Array,
    B_x: jax.Array,
    B_Lambda_re: jax.Array,
    B_Lambda_im: jax.Array,
    B_B_re: jax.Array,
    B_B_im: jax.Array,
    B_C_re: jax.Array,
    B_C_im: jax.Array,
    B_log_dt: jax.Array,
    B_Dskip: jax.Array,
    gate_w: jax.Array,
):
    del B_x
    _, S, M = A_x.shape
    Dc = A_c_kv.shape[2]
    H, D = A_w_q.shape[1], A_w_q.shape[2]
    P = B_Lambda_re.shape[0]
    assert P == M
    RC = 512
    NL = pl.cdiv(P, 128)

    hbm = pl.BlockSpec(memory_space=pltpu.HBM)
    vec = pl.BlockSpec((M,), lambda h: (0,))
    out_t = pl.pallas_call(
        functools.partial(_kernel, S=S, D=D, BQ=512, RC=RC, NH=H),
        grid=(H,),
        in_specs=[
            hbm, hbm, hbm, hbm, hbm,
            pl.BlockSpec((None, M, D), lambda h: (h, 0, 0)),
            vec, vec, hbm, hbm, hbm, hbm, vec, vec, vec,
        ],
        out_specs=hbm,
        out_shape=jax.ShapeDtypeStruct((M, S), F32),
        scratch_shapes=[
            pltpu.VMEM((M, S), BF16), pltpu.VMEM((S, M), BF16), pltpu.VMEM((S, Dc), BF16),
            pltpu.VMEM((4, M, M), BF16),
            pltpu.VMEM((2, M, D), jnp.int32), pltpu.VMEM((2, Dc, D), jnp.int32),
            pltpu.VMEM((2, Dc, D), jnp.int32),
            pltpu.VMEM((2, M, D), BF16), pltpu.VMEM((2, Dc, D), BF16),
            pltpu.VMEM((2, Dc, D), BF16),
            pltpu.VMEM((S, D), BF16), pltpu.VMEM((S, D), BF16), pltpu.VMEM((S, D), BF16),
            pltpu.VMEM((M, S), F32), pltpu.VMEM((NL, S, 128), F32), pltpu.VMEM((NL, S, 128), F32),
            pltpu.SemaphoreType.DMA((3,)), pltpu.SemaphoreType.DMA((6,)),
            pltpu.SemaphoreType.DMA((S // RC,)),
        ],
        compiler_params=pltpu.CompilerParams(
            dimension_semantics=("arbitrary",),
            vmem_limit_bytes=100 * 1024 * 1024,
        ),
    )(A_x.reshape(S, M).T, A_c_kv.reshape(S, Dc), A_w_q, A_w_uk, A_w_uv,
      jnp.swapaxes(A_w_o, 1, 2),
      B_Lambda_re, B_Lambda_im, B_B_re, B_B_im, B_C_re, B_C_im,
      B_log_dt, B_Dskip, gate_w)
    return out_t.T.reshape(1, S, M)
```
